```python
import os as _os
_os.environ.setdefault("JAX_PLATFORMS", "cpu")
import jax
import jax.numpy as jnp

def _softmax(x, axis=-1):
    return jax.nn.softmax(x, axis=axis)
def _gelu(x):
    return jax.nn.gelu(x, approximate=True)
def _silu(x):
    return jax.nn.silu(x)
def _sigmoid(x):
    return jax.nn.sigmoid(x)
def _layernorm(x, axis=-1, eps=1e-5):
    m = jnp.mean(x, axis=axis, keepdims=True)
    v = jnp.var(x, axis=axis, keepdims=True)
    return (x - m) / jnp.sqrt(v + eps)
def _scatter_add(tgt, idx, src, axis=0):
    return tgt.at[idx].add(src)
def _segment_sum(src, seg, n):
    return jax.ops.segment_sum(src, seg, n)
class _Rng:
    def __init__(self, key):
        self._k = key
    def _next(self):
        self._k, sub = jax.random.split(self._k)
        return sub
    def normal(self, shape):
        return jax.random.normal(self._next(), shape, dtype=jnp.bfloat16)
    def randint(self, lo, hi, shape):
        return jax.random.randint(self._next(), shape, lo, hi, dtype=jnp.int32)
    def uniform(self, shape, lo=0.0, hi=1.0):
        return jax.random.uniform(self._next(), shape, jnp.bfloat16, lo, hi)
    def permutation(self, n):
        return jax.random.permutation(self._next(), n)


kernel_name = 'sequential_preLN__mha_block__dense_activation_mish__prompt'

def setup_inputs():
    _rng = _Rng(jax.random.key(int.from_bytes(__import__("os").urandom(4), "little")))
    _w = (lambda a: (lambda t: t.astype(jnp.bfloat16) if jnp.issubdtype(t.dtype, jnp.floating) else t)(jnp.asarray(a)))
    def _A_setup():
        B, S, D, H = 1, 2048, 576, 32
        return {
            "x": _w((lambda *s: _rng.normal(s) * 0.05)(B, S, D)),
            "wqkv": _w((lambda *s: _rng.normal(s) * 0.05)(D, 3 * D)),
            "wo": _w((lambda *s: _rng.normal(s) * 0.05)(D, D)),
        }
    _A_in = _A_setup()

    def _B_setup():
        B, S, D, F = 1, 2048, 576, 4608
        return {
            "x": _w((lambda *s: _rng.normal(s) * 0.05)(B, S, D)),
            "w1": _w((lambda *s: _rng.normal(s) * 1.6)(D, F) * (D ** -0.5)),
            "b1": _w((lambda *s: _rng.normal(s) * 0.05)(F)),
            "w2": _w((lambda *s: _rng.normal(s) * 0.05)(F, D) * (F ** -0.5)),
        }
    _B_in = _B_setup()

    return {
        "A_x": _A_in["x"],
        "A_wqkv": _A_in["wqkv"],
        "A_wo": _A_in["wo"],
        "B_x": _B_in["x"],
        "B_w1": _B_in["w1"],
        "B_b1": _B_in["b1"],
        "B_w2": _B_in["w2"],
    }

def reference(A_x, A_wqkv, A_wo, B_x, B_w1, B_b1, B_w2):
    def _A_ref(x, wqkv, wo):
        B, S, D = x.shape
        H = 32
        Dh = D // H
        qkv = (lambda x, *d: x.transpose(*d))((x @ wqkv).reshape(B, S, 3, H, Dh), 2, 0, 3, 1, 4)
        q, k, v = qkv[0], qkv[1], qkv[2]
        scores = jnp.einsum("bhqd,bhkd->bhqk", q, k) * (Dh ** -0.5)
        p = _softmax(scores, axis=-1)
        o = jnp.einsum("bhqk,bhkd->bhqd", p, v)
        return (lambda x, *d: x.transpose(*d))(o, 0, 2, 1, 3).reshape(B, S, D) @ wo

    def _B_ref(x, w1, b1, w2):
        h = jnp.einsum("bsd,df->bsf", x, w1) + b1
        sp = jnp.log1p(jnp.exp(-jnp.abs(h))) + jnp.where(h > 0, h, jnp.zeros_like(h))
        act = h * jnp.tanh(sp)
        return jnp.einsum("bsf,fd->bsd", act, w2)

    x = A_x
    h = x + _A_ref(_layernorm(x, axis=-1), A_wqkv, A_wo)
    h2 = h + _B_ref(_layernorm(h, axis=-1), B_w1, B_b1, B_w2)
    return h2
```

```python
import functools

import numpy as np
import jax
import jax.numpy as jnp
import jax.experimental.pallas as pl
import jax.experimental.pallas.tpu as pltpu

F32 = jnp.float32
BF16 = jnp.bfloat16

S, D, H, FF = 2048, 576, 32, 4608
DH = D // H
HPT = 7
NT = 5
TW = HPT * DH
VP = 24
KB = 512
SB = 512
EPS = 1e-5
QSCALE = float(DH ** -0.5 * np.log2(np.e))
L_MIN = float(2.0 ** -40)

NN = (((1,), (0,)), ((), ()))
NTD = (((1,), (1,)), ((), ()))
TN = (((0,), (0,)), ((), ()))


def _dot(a, b, dims=NN):
    return jax.lax.dot_general(a, b, dims, preferred_element_type=F32)


def _iota(shape, dim):
    return jax.lax.broadcasted_iota(jnp.int32, shape, dim)


def _ln_t(xt):
    mu = jnp.sum(xt, axis=0, keepdims=True) * (1.0 / D)
    xc = xt - mu
    var = jnp.sum(xc * xc, axis=0, keepdims=True) * (1.0 / D)
    return xc * jax.lax.rsqrt(var + EPS)


def _mish(h):
    n = jnp.exp(jnp.minimum(h, 20.0))
    t = n * (n + 2.0)
    return h * (t / (t + 2.0))


def _kernel(xt_hbm, wqkv_hbm, wo_hbm, w1_hbm, b1_hbm, w2t_hbm, out_hbm,
            xt_v, wqkv_v, wo_v, w1_v, b1_v, w2t_v,
            xnt_s, q_s, k_s, vt_s, vh_s, m_s, attn_s, lmin_s, wo_f, wo_p, hn_s, h_s, out_v,
            sems):
    cp_x = pltpu.make_async_copy(xt_hbm, xt_v, sems.at[0])
    cp_wqkv = pltpu.make_async_copy(wqkv_hbm, wqkv_v, sems.at[1])
    cp_wo = pltpu.make_async_copy(wo_hbm, wo_v, sems.at[2])
    cp_w1 = pltpu.make_async_copy(w1_hbm, w1_v, sems.at[3])
    cp_b1 = pltpu.make_async_copy(b1_hbm, b1_v, sems.at[4])
    cp_w2 = pltpu.make_async_copy(w2t_hbm, w2t_v, sems.at[5])
    cp_x.start()
    cp_wqkv.start()
    cp_x.wait()

    for c in range(S // 512):
        xt = xt_v[:, c * 512:(c + 1) * 512].astype(F32)
        xnt_s[:, c * 512:(c + 1) * 512] = _ln_t(xt).astype(BF16)

    cp_wqkv.wait()
    cp_wo.start()
    cp_b1.start()
    cp_w1.start()
    cp_w2.start()

    lane = _iota((D, 128), 1)
    seg_r = _iota((16, 128), 0)
    seg_c = _iota((16, 128), 1)
    seg = jnp.where((seg_c >= seg_r * DH) & (seg_c < seg_r * DH + DH) & (seg_r < HPT), 1.0, 0.0).astype(BF16)

    def head_tile(col0, t):
        start = col0 + TW * t
        width = min(TW, col0 + D - start)
        a0 = (start // 128) * 128
        sh = start - a0
        lo = wqkv_v[:, a0:a0 + 128]
        if sh == 0:
            w = lo
        else:
            hi = wqkv_v[:, a0 + 128:a0 + 256]
            lo_r = pltpu.bitcast(pltpu.roll(pltpu.bitcast(lo, jnp.uint32), 128 - sh, 1), BF16)
            hi_r = pltpu.bitcast(pltpu.roll(pltpu.bitcast(hi, jnp.uint32), 128 - sh, 1), BF16)
            w = jnp.where(lane < 128 - sh, lo_r, hi_r)
        return jnp.where(lane < width, w, jnp.zeros_like(w))

    xnt = xnt_s[...]
    lane_s = _iota((S, 128), 1)
    for t in range(NT):
        qt = _dot(head_tile(0, t), xnt, TN) * QSCALE
        q_s[t] = qt.astype(BF16)
        qn2 = _dot(seg, (qt * qt).astype(BF16))
        kt = _dot(xnt, head_tile(D, t), TN)
        kn2 = _dot(seg, (kt * kt).astype(BF16), NTD)
        k_s[t] = jnp.where(lane_s == TW, 1.0, kt).astype(BF16)
        kmax2 = jnp.max(kn2, axis=1, keepdims=True)
        m_s[t] = (jnp.sqrt(qn2 * kmax2) * (-1.03125))[0:8]
    vt_s[...] = _dot(wqkv_v[:, 2 * D:3 * D], xnt, TN)

    one_row = _iota((16, S), 0) == (DH - 16)
    def vprep(g, c):
        r0 = pl.multiple_of(g * 72, 8)
        blk = vt_s[pl.ds(r0, 72), :]
        for i in range(4):
            v0 = blk[DH * i:DH * i + 16]
            v1 = blk[DH * i + 2:DH * i + 18]
            h = g * 4 + i
            vh_s[h, 0:16, :] = v0.astype(BF16)
            v1r = pltpu.roll(v1, 2, 0)
            r = _iota((16, S), 0)
            vh_s[h, 16:32, :] = jnp.where(r < 2, v1r, jnp.where(one_row, 1.0, 0.0)).astype(BF16)
        return c
    jax.lax.fori_loop(0, 8, vprep, 0)

    cp_wo.wait()
    wo_f[...] = wo_v[...].astype(F32)
    wo_p[...] = jnp.zeros_like(wo_p)
    for h in range(H):
        wo_p[VP * h:VP * h + DH, :] = wo_f[DH * h:DH * h + DH, :]

    row = _iota((128, S), 0)

    def masked_q(t, j):
        qt = q_s[t]
        lo = j * DH
        return jnp.where((row >= lo) & (row < lo + DH), qt, jnp.zeros_like(qt))

    def head_fast(h, lmin):
        t = h // HPT
        j = h - t * HPT
        negm = m_s[t, pl.ds(j, 1), :].astype(BF16)
        qm = jnp.where(row == TW, jnp.broadcast_to(negm, (128, S)), masked_q(t, j))
        acc = jnp.zeros((32, S), F32)
        for kb in range(S // KB):
            s = _dot(k_s[t, kb * KB:(kb + 1) * KB, :], qm)
            p = jnp.exp2(s).astype(BF16)
            acc = acc + _dot(vh_s[h, :, kb * KB:(kb + 1) * KB], p)
        l = acc[DH:DH + 1, :]
        attn_s[h] = acc[0:VP] * (1.0 / l)
        return jnp.minimum(lmin, l),

    def fast_body(h, lmin):
        return head_fast(h, lmin)[0]

    lmin = jax.lax.fori_loop(0, H, fast_body, jnp.full((1, S), 1.0e30, F32))
    selfeq = lmin >= L_MIN
    safe = jnp.min(jnp.where(selfeq, 1.0, 0.0)) > 0.5

    @pl.when(jnp.logical_not(safe))
    def _():
        QF = 256
        def head_slow(i, c):
            h = i // (S // QF)
            qb = i - h * (S // QF)
            q0 = pl.multiple_of(qb * QF, QF)
            t = h // HPT
            j = h - t * HPT
            rowq = _iota((128, QF), 0)
            lo = j * DH
            qt = q_s[t, :, pl.ds(q0, QF)]
            qm = jnp.where((rowq >= lo) & (rowq < lo + DH), qt, jnp.zeros_like(qt))
            def mx(kb, m):
                k0 = pl.multiple_of(kb * KB, KB)
                s = _dot(k_s[t, pl.ds(k0, KB), :], qm)
                return jnp.maximum(m, jnp.max(s, axis=0, keepdims=True))
            m = jax.lax.fori_loop(0, S // KB, mx, jnp.full((1, QF), -jnp.inf, F32))
            def pv(kb, acc):
                k0 = pl.multiple_of(kb * KB, KB)
                s = _dot(k_s[t, pl.ds(k0, KB), :], qm)
                p = jnp.exp2(s - m).astype(BF16)
                return acc + _dot(vh_s[h, :, pl.ds(k0, KB)], p)
            acc = jax.lax.fori_loop(0, S // KB, pv, jnp.zeros((32, QF), F32))
            l = acc[DH:DH + 1, :]
            attn_s[h, :, pl.ds(q0, QF)] = acc[0:VP] * (1.0 / l)
            return c
        jax.lax.fori_loop(0, H * (S // QF), head_slow, 0)

    wop = wo_p[...].astype(BF16)
    for c in range(S // 512):
        cs = slice(c * 512, (c + 1) * 512)
        a = attn_s[:, :, cs].reshape(H * VP, 512).astype(BF16)
        ht = xt_v[:, cs].astype(F32) + _dot(wop, a, TN)
        h_s[:, cs] = ht
        hn_s[:, cs] = _ln_t(ht).astype(BF16)

    cp_b1.wait()
    cp_w1.wait()
    cp_w2.wait()
    bias = b1_v[...].astype(F32).reshape(1, FF)

    def ffn(i, c):
        c0 = pl.multiple_of(i * SB, SB)
        hnt = hn_s[:, pl.ds(c0, SB)]
        h1 = _dot(hnt, w1_v[...], TN) + bias
        act = _mish(h1).astype(BF16)
        y = _dot(w2t_v[...], act, NTD)
        out_v[:, pl.ds(c0, SB)] = (h_s[:, pl.ds(c0, SB)] + y).astype(BF16)
        return c
    jax.lax.fori_loop(0, S // SB, ffn, 0)

    cp_out = pltpu.make_async_copy(out_v, out_hbm, sems.at[6])
    cp_out.start()
    cp_out.wait()


@jax.jit
def pallas_sequential_preLN__mha_block__dense_activation_mish__prompt_kernel(
    A_x: jax.Array,
    A_wqkv: jax.Array,
    A_wo: jax.Array,
    B_x: jax.Array,
    B_w1: jax.Array,
    B_b1: jax.Array,
    B_w2: jax.Array,
):
    del B_x
    xt = A_x.reshape(S, D).T
    w2t = B_w2.T
    b1 = B_b1.reshape(FF // 128, 128)
    any_spec = pl.BlockSpec(memory_space=pl.ANY)
    outt = pl.pallas_call(
        _kernel,
        out_shape=jax.ShapeDtypeStruct((D, S), BF16),
        in_specs=[any_spec] * 6,
        out_specs=any_spec,
        scratch_shapes=[
            pltpu.VMEM((D, S), BF16),
            pltpu.VMEM((D, 3 * D), BF16),
            pltpu.VMEM((D, D), BF16),
            pltpu.VMEM((D, FF), BF16),
            pltpu.VMEM((FF // 128, 128), BF16),
            pltpu.VMEM((D, FF), BF16),
            pltpu.VMEM((D, S), BF16),
            pltpu.VMEM((NT, 128, S), BF16),
            pltpu.VMEM((NT, S, 128), BF16),
            pltpu.VMEM((D, S), F32),
            pltpu.VMEM((H, 32, S), BF16),
            pltpu.VMEM((NT, 8, S), F32),
            pltpu.VMEM((H, VP, S), F32),
            pltpu.VMEM((8, 128), F32),
            pltpu.VMEM((D, D), F32),
            pltpu.VMEM((H * VP, D), F32),
            pltpu.VMEM((D, S), BF16),
            pltpu.VMEM((D, S), F32),
            pltpu.VMEM((D, S), BF16),
            pltpu.SemaphoreType.DMA((8,)),
        ],
        compiler_params=pltpu.CompilerParams(vmem_limit_bytes=120 * 1024 * 1024),
    )(xt, A_wqkv, A_wo, B_w1, b1, w2t)
    return outt.T.reshape(1, S, D)
```

```python
import numpy as np
import jax
import jax.numpy as jnp
import jax.experimental.pallas as pl
import jax.experimental.pallas.tpu as pltpu

F32 = jnp.float32
BF16 = jnp.bfloat16

S, D, H, FF = 2048, 576, 32, 4608
DH = D // H
HPT = 7
NT = 5
TW = HPT * DH
QW = NT * 128
VP = 24
CFG = dict(QB=2048, KB=128, PIPE=1, PB=512, SB=256, HU=2, NS=False)
EPS = 1e-5
QSCALE = float(DH ** -0.5 * np.log2(np.e))
L_MIN = float(2.0 ** -40)
L_MAX = float(2.0 ** 100)

NN = (((1,), (0,)), ((), ()))
NTD = (((1,), (1,)), ((), ()))
TN = (((0,), (0,)), ((), ()))


def _dot(a, b, dims=NN):
    return jax.lax.dot_general(a, b, dims, preferred_element_type=F32)


def _iota(shape, dim):
    return jax.lax.broadcasted_iota(jnp.int32, shape, dim)


def _ln_t(xt):
    mu = jnp.sum(xt, axis=0, keepdims=True) * (1.0 / D)
    xc = xt - mu
    var = jnp.sum(xc * xc, axis=0, keepdims=True) * (1.0 / D)
    return xc * jax.lax.rsqrt(var + EPS)


def _recip(d):
    r = pl.reciprocal(d, approx=True)
    return r * (2.0 - d * r)


def _mish(h):
    n = jnp.exp(jnp.minimum(h, 20.0))
    t = n * (n + 2.0)
    return (h * t) * _recip(t + 2.0)


class _NoScope:
    def __enter__(self): return self
    def __exit__(self, *a): return False


def _kernel(xt_hbm, wqkv_hbm, wo_hbm, w1_hbm, b1_hbm, w2t_hbm, out_hbm,
            xt_v, wqkv_v, wo_v, w1_v, b1_v, w2t_v,
            wqvt_s, wk_s, xnt_s, q_s, k_s, vh_s, attn_s, wo_p, wopt_s, hn_s, h_s, an_s, out_v,
            sems, xsems, osems):
    QB, KB, PIPE, PB, SB = CFG["QB"], CFG["KB"], CFG["PIPE"], CFG["PB"], CFG["SB"]
    NPB = S // PB
    NSB = S // SB
    ns = jax.named_scope if CFG["NS"] else (lambda n: _NoScope())

    def x_copy(c):
        return pltpu.make_async_copy(xt_hbm.at[:, c * PB:(c + 1) * PB], xt_v.at[:, c * PB:(c + 1) * PB], xsems.at[c])
    def w_copy(lo, hi, i):
        return pltpu.make_async_copy(wqkv_hbm.at[:, lo:hi], wqkv_v.at[:, lo:hi], sems.at[i])
    cp_wk = w_copy(512, 2 * D, 0)
    cp_wq = w_copy(0, 512, 1)
    cp_wv = w_copy(2 * D, 3 * D, 2)
    cp_wo = pltpu.make_async_copy(wo_hbm, wo_v, sems.at[3])
    cp_w1 = pltpu.make_async_copy(w1_hbm, w1_v, sems.at[4])
    cp_b1 = pltpu.make_async_copy(b1_hbm, b1_v, sems.at[5])
    cp_w2 = pltpu.make_async_copy(w2t_hbm, w2t_v, sems.at[6])

    lane = _iota((D, 128), 1)

    def head_tile(col0, t):
        start = col0 + TW * t
        width = min(TW, col0 + D - start)
        a0 = (start // 128) * 128
        sh = start - a0
        lo = wqkv_v[:, a0:a0 + 128]
        if sh == 0:
            w = lo
        else:
            hi = wqkv_v[:, a0 + 128:a0 + 256]
            both = jnp.where(lane >= sh, lo, hi)
            w = pltpu.bitcast(pltpu.roll(pltpu.bitcast(both, jnp.uint32), 128 - sh, 1), BF16)
        return jnp.where(lane < width, w, jnp.zeros_like(w))

    def ln1(c):
        LW = CFG.get("LW", 256)
        cols = []
        for i in range(PB // LW):
            cs = slice(c * PB + i * LW, c * PB + (i + 1) * LW)
            xnt = _ln_t(xt_v[:, cs].astype(F32)).astype(BF16)
            xnt_s[:, cs] = xnt
            cols.append(xnt if CFG.get("KTN", 0) else xnt.T)
        return jnp.concatenate(cols, axis=1 if CFG.get("KTN", 0) else 0)

    def kmm(xn):
        return _dot(xn, wk_s[...], TN) if CFG.get("KTN", 0) else _dot(xn,  wk_s[...])

    x_copy(0).start()
    cp_wk.start()
    x_copy(1).start()
    def zero_q(t, c):
        for j in range(HPT):
            r0 = (DH * j) // 16 * 16
            if r0 > 0:
                q_s[HPT * t + j, 0:r0, :] = jnp.zeros((r0, S), BF16)
            if r0 + 32 < 128:
                q_s[HPT * t + j, r0 + 32:128, :] = jnp.zeros((128 - r0 - 32, S), BF16)
        return c

    with ns("pro"):
        jax.lax.fori_loop(0, NT, zero_q, 0)
        x_copy(0).wait()
        xn = ln1(0)
        cp_wk.wait()
        x_copy(1).wait()
        x_copy(2).start()
        x_copy(3).start()
        cp_wo.start()
        for t in range(NT):
            wk_s[:, t * 128:(t + 1) * 128] = head_tile(D, t)
    def k_finish(c, kt):
        for t in range(NT):
            k_s[t, c * PB:(c + 1) * PB, :] = kt[:, t * 128:(t + 1) * 128].astype(BF16)

    def wo_prep():
        zpad = jnp.zeros((VP - DH, D), F32)
        for g in range(4):
            wblk = wo_v[144 * g:144 * (g + 1), :].astype(F32)
            pieces = []
            for i in range(8):
                pieces += [wblk[DH * i:DH * i + DH], zpad]
            wo_p[192 * g:192 * (g + 1), :] = jnp.concatenate(pieces, axis=0).astype(BF16)
        wopt_s[...] = wo_p[...].T

    with ns("loopA"):
        xn0 = xn
        xn = ln1(1)
        kt0 = kmm(xn0)
        x_copy(2).wait()
        x_copy(3).wait()
        cp_wo.wait()
        cp_wq.start()
        cp_wv.start()
        xn1 = xn
        xn = ln1(2)
        kt1 = kmm(xn1)
        k_finish(0, kt0)
        wo_prep()
        cp_wq.wait()
        cp_wv.wait()
        cp_b1.start()
        cp_w1.start()
        cp_w2.start()
        xn2 = xn
        xn = ln1(3)
        kt2 = kmm(xn2)
        k_finish(1, kt1)
        for t in range(NT):
            wqvt_s[t * 128:(t + 1) * 128, :] = head_tile(0, t).T
        kt3 = kmm(xn)
        wqvt_s[QW:QW + D, :] = wqkv_v[:, 2 * D:3 * D].T
        k_finish(2, kt2)
        k_finish(3, kt3)

    def qv_body(c, carry):
        cs = pl.ds(pl.multiple_of(c * PB, PB), PB)
        xnt = xnt_s[:, cs]
        q = _dot(wqvt_s[0:QW, :], xnt) * QSCALE
        v_all = _dot(wqvt_s[QW:QW + D, :], xnt)
        for t in range(NT):
            for j in range(min(HPT, H - HPT * t)):
                r0 = (DH * j) // 16 * 16
                rr = _iota((32, PB), 0) + r0
                blk = q[t * 128 + r0:t * 128 + r0 + 32]
                q_s[HPT * t + j, r0:r0 + 32, cs] = jnp.where((rr >= DH * j) & (rr < DH * j + DH), blk, 0.0).astype(BF16)
        r24 = _iota((VP, PB), 0)
        ones_row = jnp.where(r24 == DH, 1.0, 0.0)
        for h in range(H):
            r0 = DH * h
            if r0 + VP <= D:
                v = v_all[r0:r0 + VP]
            else:
                v = pltpu.roll(v_all[D - VP:D], VP - (r0 - (D - VP)), 0)
            vh_s[h, :, cs] = jnp.where(r24 < DH, v, ones_row)
        if CFG.get("BV", 0) == 2:
            for t in range(NT):
                q_store(t, negms[t])
        return carry

    with ns("loopB"):
        jax.lax.fori_loop(0, NPB, qv_body, 0)

    row = _iota((128, QB), 0)
    nq, nk = S // QB, S // KB
    steps = [(qb, kb) for qb in range(nq) for kb in range(nk)]

    def head_fast(h, carry):
        lmin, lmax, t, j = carry
        def qk(st):
            qb, kb = st
            return _dot(k_s[t, kb * KB:(kb + 1) * KB, :], q_s[h, :, qb * QB:(qb + 1) * QB])
        pend = [qk(steps[i]) for i in range(PIPE)]
        acc = None
        for i, (qb, kb) in enumerate(steps):
            if i + PIPE < len(steps):
                pend.append(qk(steps[i + PIPE]))
            p = jnp.exp2(pend.pop(0)).astype(BF16)
            y = _dot(vh_s[h, :, kb * KB:(kb + 1) * KB], p)
            acc = y if kb == 0 else acc + y
            if kb == nk - 1:
                attn_s[h, :, qb * QB:(qb + 1) * QB] = acc
                lmin = jnp.minimum(lmin, acc[DH:DH + 1, :])
                lmax = jnp.maximum(lmax, acc[DH:DH + 1, :])
        wrap = j == HPT - 1
        return lmin, lmax, jnp.where(wrap, t + 1, t), jnp.where(wrap, 0, j + 1)

    with ns("attn"):
        lmin, lmax, _, _ = jax.lax.fori_loop(0, H, head_fast, (jnp.ones((1, QB), F32), jnp.ones((1, QB), F32), jnp.int32(0), jnp.int32(0)),
                                       unroll=CFG["HU"])
    safe = jnp.min(jnp.where((lmin >= L_MIN) & (lmax <= L_MAX), 1.0, 0.0)) > 0.5

    @pl.when(jnp.logical_not(safe))
    def _():
        QF, KF = 256, 512
        def head_slow(i, c):
            h = i // (S // QF)
            qb = i - h * (S // QF)
            q0 = pl.multiple_of(qb * QF, QF)
            t = h // HPT
            j = h - t * HPT
            qm = q_s[h, :, pl.ds(q0, QF)]
            def mx(kb, m):
                k0 = pl.multiple_of(kb * KF, KF)
                s = _dot(k_s[t, pl.ds(k0, KF), :], qm)
                return jnp.maximum(m, jnp.max(s, axis=0, keepdims=True))
            m = jax.lax.fori_loop(0, S // KF, mx, jnp.full((1, QF), -jnp.inf, F32))
            def pv(kb, acc):
                k0 = pl.multiple_of(kb * KF, KF)
                s = _dot(k_s[t, pl.ds(k0, KF), :], qm)
                p = jnp.exp2(s - m).astype(BF16)
                return acc + _dot(vh_s[h, :, pl.ds(k0, KF)], p)
            acc = jax.lax.fori_loop(0, S // KF, pv, jnp.zeros((VP, QF), F32))
            attn_s[h, :, pl.ds(q0, QF)] = acc
            return c
        jax.lax.fori_loop(0, H * (S // QF), head_slow, 0)

    OB = CFG.get("OB", 512)

    def a_norm(i):
        cs = pl.ds(i * OB if isinstance(i, int) else pl.multiple_of(i * OB, OB), OB)
        a = attn_s[:, :, cs]
        return (a * _recip(a[:, DH:DH + 1, :])).reshape(H * VP, OB).astype(BF16)

    def ln2(i, slot):
        cs = pl.ds(i * SB if isinstance(i, int) else pl.multiple_of(i * SB, SB), SB)
        hn_s[slot] = _ln_t(h_s[:, cs]).astype(BF16).T

    def oproj(i, c):
        cs = pl.ds(pl.multiple_of(i * OB, OB), OB)
        if CFG.get("OP", 0):
            a = an_s[...]
            nxt = a_norm(jnp.minimum(i + 1, S // OB - 1))
            h_s[:, cs] = xt_v[:, cs].astype(F32) + _dot(wopt_s[...], a)
            an_s[...] = nxt
        else:
            h_s[:, cs] = xt_v[:, cs].astype(F32) + _dot(wopt_s[...], a_norm(i))
        return c

    def out_copy(i):
        c0 = i * SB if isinstance(i, int) else pl.multiple_of(i * SB, SB)
        return pltpu.make_async_copy(out_v.at[:, pl.ds(c0, SB)], out_hbm.at[:, pl.ds(c0, SB)], osems.at[i])

    with ns("oproj0"):
        if CFG.get("OP", 0):
            an_s[...] = a_norm(0)
        jax.lax.fori_loop(0, S // OB, oproj, 0)
        ln2(0, 0)
        cp_b1.wait()
        cp_w1.wait()
        cp_w2.wait()
    bias = b1_v[...].astype(F32).reshape(1, FF)

    def ffn(i, c):
        slot = i % 2
        c0 = pl.multiple_of(i * SB, SB)
        h1 = _dot(hn_s[slot], w1_v[...]) + bias
        ln2(jnp.minimum(i + 1, NSB - 1), 1 - slot)
        act = _mish(h1).astype(BF16)
        y = _dot(w2t_v[...], act, NTD)
        out_v[:, pl.ds(c0, SB)] = (h_s[:, pl.ds(c0, SB)] + y).astype(BF16)
        out_copy(i).start()
        return c
    with ns("ffn"):
        jax.lax.fori_loop(0, NSB, ffn, 0)
    with ns("outdma"):
        for i in range(NSB):
            out_copy(i).wait()


def build(x, wqkv, wo, w1, b1, w2):
    PB, SB = CFG["PB"], CFG["SB"]
    xt = x.reshape(S, D).T
    w2t = w2.T
    b1 = b1.reshape(FF // 128, 128)
    any_spec = pl.BlockSpec(memory_space=pl.ANY)
    outt = pl.pallas_call(
        _kernel,
        out_shape=jax.ShapeDtypeStruct((D, S), BF16),
        in_specs=[any_spec] * 6,
        out_specs=any_spec,
        scratch_shapes=[
            pltpu.VMEM((D, S), BF16),
            pltpu.VMEM((D, 3 * D), BF16),
            pltpu.VMEM((D, D), BF16),
            pltpu.VMEM((D, FF), BF16),
            pltpu.VMEM((FF // 128, 128), BF16),
            pltpu.VMEM((D, FF), BF16),
            pltpu.VMEM((QW + D, D), BF16),
            pltpu.VMEM((D, QW), BF16),
            pltpu.VMEM((D, S), BF16),
            pltpu.VMEM((NT * HPT, 128, S), BF16),
            pltpu.VMEM((NT, S, 128), BF16),
            pltpu.VMEM((H, VP, S), F32),
            pltpu.VMEM((H, VP, S), F32),
            pltpu.VMEM((H * VP, D), BF16),
            pltpu.VMEM((D, H * VP), BF16),
            pltpu.VMEM((2, SB, D), BF16),
            pltpu.VMEM((D, S), F32),
            pltpu.VMEM((H * VP, CFG.get("OB", 512)), BF16),
            pltpu.VMEM((D, S), BF16),
            pltpu.SemaphoreType.DMA((8,)),
            pltpu.SemaphoreType.DMA((16,)),
            pltpu.SemaphoreType.DMA((16,)),
        ],
        compiler_params=pltpu.CompilerParams(vmem_limit_bytes=120 * 1024 * 1024, flags=CFG.get('FLAGS')),
    )(xt, wqkv, wo, w1, b1, w2t)
    return outt.T.reshape(1, S, D)


@jax.jit
def pallas_sequential_preLN__mha_block__dense_activation_mish__prompt_kernel(A_x, A_wqkv, A_wo, B_x, B_w1, B_b1, B_w2):
    return build(A_x, A_wqkv, A_wo, B_w1, B_b1, B_w2)
```

```python
import numpy as np
import jax
import jax.numpy as jnp
import jax.experimental.pallas as pl
import jax.experimental.pallas.tpu as pltpu

F32 = jnp.float32
BF16 = jnp.bfloat16

S, D, H, FF = 2048, 576, 32, 4608
DH = D // H
HPT = 7
NT = 5
TW = HPT * DH
QR = 4 * 128 + 80
VP = 24
KB = 128
PB = 512
OB = 512
SB = 256
EPS = 1e-5
QSCALE = float(DH ** -0.5 * np.log2(np.e))
L_MIN = float(2.0 ** -60)
L_MAX = float(2.0 ** 60)

NN = (((1,), (0,)), ((), ()))
NT_DIMS = (((1,), (1,)), ((), ()))


def _dot(a, b, dims=NN):
    return jax.lax.dot_general(a, b, dims, preferred_element_type=F32)


def _iota(shape, dim):
    return jax.lax.broadcasted_iota(jnp.int32, shape, dim)


def _ln_t(xt):
    mu = jnp.sum(xt, axis=0, keepdims=True) * (1.0 / D)
    xc = xt - mu
    var = jnp.sum(xc * xc, axis=0, keepdims=True) * (1.0 / D)
    return xc * jax.lax.rsqrt(var + EPS)


def _recip(d):
    r = pl.reciprocal(d, approx=True)
    return r * (2.0 - d * r)


def _mish(h):
    n = jnp.exp(jnp.minimum(h, 20.0))
    t = n * (n + 2.0)
    return h * (t * _recip(t + 2.0))


def _kernel(xt_hbm, wqkv_hbm, wo_hbm, w1_hbm, b1_hbm, w2t_hbm, out_hbm,
            xt_v, wqkv_v, wo_v, w1_v, b1_v, w2t_v,
            wqvt_s, wk_s, wot_s, xnt_s, q_s, k_s, v_s, attn_s, h_s, hn_s, out_v,
            wsems, xsems, osems):
    def x_copy(c):
        cols = slice(c * PB, (c + 1) * PB)
        return pltpu.make_async_copy(xt_hbm.at[:, cols], xt_v.at[:, cols], xsems.at[c])

    def wqkv_copy(lo, hi, i):
        return pltpu.make_async_copy(wqkv_hbm.at[:, lo:hi], wqkv_v.at[:, lo:hi], wsems.at[i])

    cp_wk = wqkv_copy(512, 2 * D, 0)
    cp_wq = wqkv_copy(0, 512, 1)
    cp_wv = wqkv_copy(2 * D, 3 * D, 2)
    cp_wo = pltpu.make_async_copy(wo_hbm, wo_v, wsems.at[3])
    cp_w1 = pltpu.make_async_copy(w1_hbm, w1_v, wsems.at[4])
    cp_b1 = pltpu.make_async_copy(b1_hbm, b1_v, wsems.at[5])
    cp_w2 = pltpu.make_async_copy(w2t_hbm, w2t_v, wsems.at[6])

    lane = _iota((D, 128), 1)

    def head_tile(col0, t):
        start = col0 + TW * t
        width = min(TW, col0 + D - start)
        a0 = start // 128 * 128
        sh = start - a0
        w = wqkv_v[:, a0:a0 + 128]
        if sh + width > 128:
            w = jnp.where(lane >= sh, w, wqkv_v[:, a0 + 128:a0 + 256])
        if sh:
            w = pltpu.bitcast(pltpu.roll(pltpu.bitcast(w, jnp.uint32), 128 - sh, 1), BF16)
        return jnp.where(lane < width, w, jnp.zeros_like(w))

    def ln1(c):
        parts = []
        for i in range(PB // 256):
            cols = slice(c * PB + i * 256, c * PB + (i + 1) * 256)
            xnt = _ln_t(xt_v[:, cols].astype(F32)).astype(BF16)
            xnt_s[:, cols] = xnt
            parts.append(xnt.T)
        return jnp.concatenate(parts, axis=0)

    def k_store(c, k):
        for t in range(NT):
            k_s[t, c * PB:(c + 1) * PB, :] = k[:, t * 128:(t + 1) * 128].astype(BF16)

    def head_rows(j):
        return DH * j // 16 * 16

    def zero_q(t, heads):
        for j in range(heads):
            r0 = head_rows(j)
            if r0 > 0:
                q_s[HPT * t + j, 0:r0, :] = jnp.zeros((r0, S), BF16)
            if r0 + 32 < 128:
                q_s[HPT * t + j, r0 + 32:128, :] = jnp.zeros((96 - r0, S), BF16)

    x_copy(0).start()
    cp_wk.start()
    x_copy(1).start()
    pl.loop(0, NT - 1)(lambda t: zero_q(t, HPT))
    zero_q(NT - 1, H - HPT * (NT - 1))
    x_copy(0).wait()
    xn0 = ln1(0)
    cp_wk.wait()
    x_copy(1).wait()
    x_copy(2).start()
    x_copy(3).start()
    cp_wo.start()
    for t in range(NT):
        wk_s[:, t * 128:(t + 1) * 128] = head_tile(D, t)
    xn1 = ln1(1)
    k0 = _dot(xn0, wk_s[...])
    x_copy(2).wait()
    x_copy(3).wait()
    cp_wo.wait()
    cp_wq.start()
    cp_wv.start()
    xn2 = ln1(2)
    k1 = _dot(xn1, wk_s[...])
    k_store(0, k0)
    wot_s[...] = wo_v[...].T
    cp_wq.wait()
    cp_wv.wait()
    cp_b1.start()
    cp_w1.start()
    cp_w2.start()
    xn3 = ln1(3)
    k2 = _dot(xn2, wk_s[...])
    k_store(1, k1)
    for t in range(NT - 1):
        wqvt_s[t * 128:(t + 1) * 128, :] = head_tile(0, t).T
    wqvt_s[(NT - 1) * 128:QR, :] = head_tile(0, NT - 1).T[0:QR - (NT - 1) * 128]
    k3 = _dot(xn3, wk_s[...])
    wqvt_s[QR:QR + D, :] = wqkv_v[:, 2 * D:3 * D].T
    k_store(2, k2)
    k_store(3, k3)

    def qv_block(c):
        cols = pl.ds(pl.multiple_of(c * PB, PB), PB)
        qv = _dot(wqvt_s[...], xnt_s[:, cols])
        q = qv[0:QR] * QSCALE
        v = qv[QR:QR + D]
        for h in range(H):
            t, j = divmod(h, HPT)
            r0 = head_rows(j)
            rows = _iota((32, PB), 0) + r0
            blk = q[t * 128 + r0:t * 128 + r0 + 32]
            q_s[h, r0:r0 + 32, cols] = jnp.where((rows >= DH * j) & (rows < DH * (j + 1)), blk, 0.0).astype(BF16)
        r24 = _iota((VP, PB), 0)
        ones_row = jnp.where(r24 == DH, 1.0, 0.0)
        for h in range(H):
            r0 = DH * h
            if r0 + VP <= D:
                vh = v[r0:r0 + VP]
            else:
                vh = pltpu.roll(v[D - VP:D], D - r0, 0)
            v_s[h, :, cols] = jnp.where(r24 < DH, vh, ones_row)

    pl.loop(0, S // PB)(qv_block)

    def heads(i, carry):
        lmin, lmax, t, j = carry
        for u in range(2):
            h = 2 * i + u
            qm = q_s[h]
            s_cur = _dot(k_s[t, 0:KB, :], qm)
            acc = None
            for kb in range(S // KB):
                if kb + 1 < S // KB:
                    s_nxt = _dot(k_s[t, (kb + 1) * KB:(kb + 2) * KB, :], qm)
                y = _dot(v_s[h, :, kb * KB:(kb + 1) * KB], jnp.exp2(s_cur).astype(BF16))
                acc = y if kb == 0 else acc + y
                s_cur = s_nxt
            attn_s[h] = acc
            l = acc[DH:DH + 1, :]
            lmin, lmax = jnp.minimum(lmin, l), jnp.maximum(lmax, l)
            wrap = j == HPT - 1
            t, j = jnp.where(wrap, t + 1, t), jnp.where(wrap, 0, j + 1)
        return lmin, lmax, t, j

    one = jnp.ones((1, S), F32)
    lmin, lmax, _, _ = jax.lax.fori_loop(0, H // 2, heads, (one, one, jnp.int32(0), jnp.int32(0)))
    in_range = (lmin >= L_MIN) & (lmax <= L_MAX)
    safe = jnp.min(jnp.where(in_range, 1.0, 0.0)) > 0.5

    @pl.when(jnp.logical_not(safe))
    def _():
        QF, KF = 256, 512

        def head_block(i):
            h = i // (S // QF)
            cols = pl.ds(pl.multiple_of((i - h * (S // QF)) * QF, QF), QF)
            t = h // HPT
            qm = q_s[h, :, cols]

            def keys(kb):
                return pl.ds(pl.multiple_of(kb * KF, KF), KF)

            def row_max(kb, m):
                return jnp.maximum(m, jnp.max(_dot(k_s[t, keys(kb), :], qm), axis=0, keepdims=True))
            m = jax.lax.fori_loop(0, S // KF, row_max, jnp.full((1, QF), -jnp.inf, F32))

            def accumulate(kb, acc):
                p = jnp.exp2(_dot(k_s[t, keys(kb), :], qm) - m).astype(BF16)
                return acc + _dot(v_s[h, :, keys(kb)], p)
            attn_s[h, :, cols] = jax.lax.fori_loop(0, S // KF, accumulate, jnp.zeros((VP, QF), F32))

        pl.loop(0, H * (S // QF))(head_block)

    def oproj(i):
        cols = pl.ds(pl.multiple_of(i * OB, OB), OB)
        a = attn_s[:, :, cols]
        a = a * _recip(a[:, DH:DH + 1, :])
        a = jnp.concatenate([a[h, 0:DH] for h in range(H)], axis=0).astype(BF16)
        h_s[:, cols] = xt_v[:, cols].astype(F32) + _dot(wot_s[...], a)

    def ln2(i, slot):
        cols = pl.ds(i * SB if isinstance(i, int) else pl.multiple_of(i * SB, SB), SB)
        hn_s[slot] = _ln_t(h_s[:, cols]).astype(BF16).T

    pl.loop(0, S // OB)(oproj)
    ln2(0, 0)
    cp_b1.wait()
    cp_w1.wait()
    cp_w2.wait()
    bias = b1_v[...].astype(F32).reshape(1, FF)

    def out_copy(i):
        cols = pl.ds(i * SB if isinstance(i, int) else pl.multiple_of(i * SB, SB), SB)
        return pltpu.make_async_copy(out_v.at[:, cols], out_hbm.at[:, cols], osems.at[i])

    def ffn(i):
        slot = i % 2
        cols = pl.ds(pl.multiple_of(i * SB, SB), SB)
        h1 = _dot(hn_s[slot], w1_v[...]) + bias
        ln2(jnp.minimum(i + 1, S // SB - 1), 1 - slot)
        y = _dot(w2t_v[...], _mish(h1).astype(BF16), NT_DIMS)
        out_v[:, cols] = (h_s[:, cols] + y).astype(BF16)
        out_copy(i).start()

    pl.loop(0, S // SB)(ffn)
    for i in range(S // SB):
        out_copy(i).wait()


@jax.jit
def pallas_sequential_preLN__mha_block__dense_activation_mish__prompt_kernel(
    A_x: jax.Array,
    A_wqkv: jax.Array,
    A_wo: jax.Array,
    B_x: jax.Array,
    B_w1: jax.Array,
    B_b1: jax.Array,
    B_w2: jax.Array,
):
    del B_x
    any_spec = pl.BlockSpec(memory_space=pl.ANY)
    out_t = pl.pallas_call(
        _kernel,
        out_shape=jax.ShapeDtypeStruct((D, S), BF16),
        in_specs=[any_spec] * 6,
        out_specs=any_spec,
        scratch_shapes=[
            pltpu.VMEM((D, S), BF16),
            pltpu.VMEM((D, 3 * D), BF16),
            pltpu.VMEM((D, D), BF16),
            pltpu.VMEM((D, FF), BF16),
            pltpu.VMEM((FF // 128, 128), BF16),
            pltpu.VMEM((D, FF), BF16),
            pltpu.VMEM((QR + D, D), BF16),
            pltpu.VMEM((D, NT * 128), BF16),
            pltpu.VMEM((D, D), BF16),
            pltpu.VMEM((D, S), BF16),
            pltpu.VMEM((H, 128, S), BF16),
            pltpu.VMEM((NT, S, 128), BF16),
            pltpu.VMEM((H, VP, S), F32),
            pltpu.VMEM((H, VP, S), F32),
            pltpu.VMEM((D, S), F32),
            pltpu.VMEM((2, SB, D), BF16),
            pltpu.VMEM((D, S), BF16),
            pltpu.SemaphoreType.DMA((7,)),
            pltpu.SemaphoreType.DMA((S // PB,)),
            pltpu.SemaphoreType.DMA((S // SB,)),
        ],
        compiler_params=pltpu.CompilerParams(vmem_limit_bytes=100 * 1024 * 1024),
    )(A_x.reshape(S, D).T, A_wqkv, A_wo, B_w1, B_b1.reshape(FF // 128, 128), B_w2.T)
    return out_t.T.reshape(1, S, D)
```
